```python
import os as _os
_os.environ.setdefault("JAX_PLATFORMS", "cpu")
import jax
import jax.numpy as jnp

def _softmax(x, axis=-1):
    return jax.nn.softmax(x, axis=axis)
def _gelu(x):
    return jax.nn.gelu(x, approximate=True)
def _silu(x):
    return jax.nn.silu(x)
def _sigmoid(x):
    return jax.nn.sigmoid(x)
def _layernorm(x, axis=-1, eps=1e-5):
    m = jnp.mean(x, axis=axis, keepdims=True)
    v = jnp.var(x, axis=axis, keepdims=True)
    return (x - m) / jnp.sqrt(v + eps)
def _scatter_add(tgt, idx, src, axis=0):
    return tgt.at[idx].add(src)
def _segment_sum(src, seg, n):
    return jax.ops.segment_sum(src, seg, n)
class _Rng:
    def __init__(self, key):
        self._k = key
    def _next(self):
        self._k, sub = jax.random.split(self._k)
        return sub
    def normal(self, shape):
        return jax.random.normal(self._next(), shape, dtype=jnp.bfloat16)
    def randint(self, lo, hi, shape):
        return jax.random.randint(self._next(), shape, lo, hi, dtype=jnp.int32)
    def uniform(self, shape, lo=0.0, hi=1.0):
        return jax.random.uniform(self._next(), shape, jnp.bfloat16, lo, hi)
    def permutation(self, n):
        return jax.random.permutation(self._next(), n)


kernel_name = 'standalone__geglu_ffn__prompt'

def setup_inputs():
    _rng = _Rng(jax.random.key(int.from_bytes(__import__("os").urandom(4), "little")))
    _w = (lambda a: (lambda t: t.astype(jnp.bfloat16) if jnp.issubdtype(t.dtype, jnp.floating) else t)(jnp.asarray(a)))
    B, S, D, F = 1, 2048, 576, 4608
    return {
        "x": _w((lambda *s: _rng.normal(s) * 0.05)(B, S, D)),
        "w_gate": _w((lambda *s: _rng.normal(s) * 0.05)(D, F)),
        "w_up": _w((lambda *s: _rng.normal(s) * 0.05)(D, F)),
        "w_down": _w((lambda *s: _rng.normal(s) * 0.05)(F, D)),
    }

def reference(x, w_gate, w_up, w_down):
    return (_gelu(x @ w_gate) * (x @ w_up)) @ w_down
```

```python
import jax
import jax.numpy as jnp
from jax import lax
import jax.experimental.pallas as pl
import jax.experimental.pallas.tpu as pltpu

_C0 = 0.7978845608028654
_C1 = 0.7978845608028654 * 0.044715

_BF = 512
_SM = 512
_GW = 256


def _geglu(g, u):
    t = jnp.tanh(g * (_C0 + _C1 * (g * g)))
    return (g * u) * (0.5 + 0.5 * t)


@jax.jit
def pallas_standalone__geglu_ffn__prompt_kernel(
    x: jax.Array,
    w_gate: jax.Array,
    w_up: jax.Array,
    w_down: jax.Array,
):
    B, S0, D = x.shape
    S = B * S0
    F = w_gate.shape[1]
    bf16, f32 = jnp.bfloat16, jnp.float32
    nf, nc = F // _BF, _BF // _GW
    assert (S, nc) == (2048, 2) and F % _BF == 0
    xp, xo = (256, 256, 512, 1024), (0, 256, 512, 1024)
    op, oo = (512, 512, 512, 256, 256), (0, 512, 1024, 1536, 1792)

    def kernel(xT_hbm, wg_hbm, wu_hbm, wdT_hbm, o_hbm,
               xT_v, x_v, wg_v, wu_v, wd_v, h_v, acc_v, o_v,
               xsem, psem, gsem, usem, dsem, osem):
        def xcopy(i):
            s = pl.ds(xo[i], xp[i])
            return pltpu.make_async_copy(xT_hbm.at[:, s], xT_v.at[:, s], xsem.at[i])

        def wcopy(hbm, v, sem, j):
            s = pl.ds(pl.multiple_of(j * _BF, _BF), _BF)
            return pltpu.make_async_copy(hbm.at[:, s], v.at[j], sem.at[j])

        def pcopy(c):
            s = pl.ds(c * _GW, _GW)
            return (pltpu.make_async_copy(wg_hbm.at[:, s], wg_v.at[0, :, s], psem.at[2 * c]),
                    pltpu.make_async_copy(wu_hbm.at[:, s], wu_v.at[0, :, s], psem.at[2 * c + 1]))

        def ocopy(i):
            s = pl.ds(oo[i], op[i])
            return pltpu.make_async_copy(o_v.at[:, s], o_hbm.at[:, s], osem.at[i])

        def up(j, r0, n, c):
            cs = slice(c * _GW, (c + 1) * _GW)
            w = jnp.concatenate([wg_v[j, :, cs], wu_v[j, :, cs]], axis=1)
            gu = jnp.dot(x_v[r0:r0 + n, :], w, preferred_element_type=f32)
            h_v[r0:r0 + n, cs] = _geglu(gu[:, :_GW], gu[:, _GW:]).astype(bf16)

        def down(j, r0, n):
            return lax.dot_general(wd_v[j], h_v[r0:r0 + n, :], (((1,), (1,)), ((), ())),
                                   preferred_element_type=f32)

        def transpose(r0, n):
            x_v[r0:r0 + n, :] = xT_v[:, r0:r0 + n].T

        xcopy(0).start()
        for cp in pcopy(0):
            cp.start()
        acc_v[...] = jnp.zeros_like(acc_v)
        xcopy(0).wait()
        xcopy(1).start()
        transpose(0, 256)
        for cp in pcopy(0):
            cp.wait()
        for cp in pcopy(1):
            cp.start()
        up(0, 0, 192, 0)
        xcopy(1).wait()
        xcopy(2).start()
        up(0, 192, 64, 0)
        transpose(256, 256)
        up(0, 256, 256, 0)
        for cp in pcopy(1):
            cp.wait()
        xcopy(2).wait()
        xcopy(3).start()
        up(0, 0, 512, 1)
        transpose(512, 512)
        up(0, 512, 512, 0)
        up(0, 512, 384, 1)
        xcopy(3).wait()
        wcopy(wdT_hbm, wd_v, dsem, 0).start()
        wcopy(wg_hbm, wg_v, gsem, 1).start()
        wcopy(wu_hbm, wu_v, usem, 1).start()
        up(0, 896, 128, 1)
        transpose(1024, 256)
        transpose(1280, 256)
        up(0, 1024, 256, 0)
        transpose(1536, 512)
        up(0, 1024, 256, 1)
        for r0, n in ((1280, 256), (1536, 512)):
            for c in range(nc):
                up(0, r0, n, c)

        def body(j, carry):
            wcopy(wdT_hbm, wd_v, dsem, j - 1).wait()
            wcopy(wg_hbm, wg_v, gsem, j).wait()
            wcopy(wu_hbm, wu_v, usem, j).wait()
            wcopy(wdT_hbm, wd_v, dsem, j).start()

            @pl.when(j + 1 < nf)
            def _():
                jn = jnp.minimum(j + 1, nf - 1)
                wcopy(wg_hbm, wg_v, gsem, jn).start()
                wcopy(wu_hbm, wu_v, usem, jn).start()

            for r0 in range(0, S, _SM):
                acc_v[:, r0:r0 + _SM] += down(j - 1, r0, _SM)
                for c in range(nc):
                    up(j, r0, _SM, c)
            return carry

        lax.fori_loop(1, nf, body, 0)

        wcopy(wdT_hbm, wd_v, dsem, nf - 1).wait()
        for i in range(len(op)):
            r0, n = oo[i], op[i]
            o_v[:, r0:r0 + n] = (acc_v[:, r0:r0 + n] + down(nf - 1, r0, n)).astype(o_v.dtype)
            ocopy(i).start()
        for i in range(len(op)):
            ocopy(i).wait()

    any_spec = pl.BlockSpec(memory_space=pl.ANY)
    dma = pltpu.SemaphoreType.DMA
    oT = pl.pallas_call(
        kernel,
        in_specs=[any_spec] * 4,
        out_specs=any_spec,
        out_shape=jax.ShapeDtypeStruct((D, S), x.dtype),
        scratch_shapes=[
            pltpu.VMEM((D, S), bf16), pltpu.VMEM((S, D), bf16),
            pltpu.VMEM((nf, D, _BF), bf16), pltpu.VMEM((nf, D, _BF), bf16),
            pltpu.VMEM((nf, D, _BF), bf16),
            pltpu.VMEM((S, _BF), bf16), pltpu.VMEM((D, S), f32), pltpu.VMEM((D, S), x.dtype),
            dma((len(xp),)), dma((2 * nc,)), dma((nf,)), dma((nf,)), dma((nf,)), dma((len(op),)),
        ],
        compiler_params=pltpu.CompilerParams(vmem_limit_bytes=100 * 1024 * 1024),
    )(x.reshape(S, D).T, w_gate, w_up, w_down.T)
    return oT.T.reshape(B, S0, D)
```

```python
import jax
import jax.numpy as jnp
from jax import lax
import jax.experimental.pallas as pl
import jax.experimental.pallas.tpu as pltpu

_C0 = 0.7978845608028654
_C1 = 0.7978845608028654 * 0.044715

_BF = 512
_GW = 256
_SM = 512
_RV = 416
_X_PIECES = ((0, 256), (256, 384), (640, 128), (768, 1280))
_O_PIECES = ((0, 512), (512, 512), (1024, 512), (1536, 256), (1792, 128), (1920, 128))


def _twice_geglu(g, u):
    t = jnp.tanh(g * (_C0 + _C1 * (g * g)))
    return (g * (1.0 + t)) * u


@jax.jit
def pallas_standalone__geglu_ffn__prompt_kernel(
    x: jax.Array,
    w_gate: jax.Array,
    w_up: jax.Array,
    w_down: jax.Array,
):
    B, S0, D = x.shape
    S = B * S0
    F = w_gate.shape[1]
    bf16, f32, u32, i32 = jnp.bfloat16, jnp.float32, jnp.uint32, jnp.int32
    nf, nc = F // _BF, _BF // _GW
    KM = D // 128 * 128
    KT = D - KM
    assert S == 2048 and F % _BF == 0 and nf >= 2 and KT > 0 and D % 16 == 0
    assert x.dtype == w_gate.dtype == w_up.dtype == w_down.dtype == bf16

    def kernel(xT_hbm, wg_hbm, wu_hbm, wdT_hbm, oT_hbm,
               xT_v, x_v, w_v, h_v, acc_v, o_v, xb_v, wb_v, tail_v, zero_v,
               xsem, psem, wsem, osem):

        def x_copy(i):
            s = pl.ds(*_X_PIECES[i])
            return pltpu.make_async_copy(xT_hbm.at[:, s], xT_v.at[:, s], xsem)

        def first_copies(c):
            s = pl.ds(c * _GW, _GW)
            return [pltpu.make_async_copy(src.at[:, s], w_v.at[0, k, :, s], psem)
                    for k, src in enumerate((wg_hbm, wu_hbm))]

        def group_copies(j, j_up):
            return [pltpu.make_async_copy(
                src.at[:, pl.ds(pl.multiple_of(jj * _BF, _BF), _BF)], w_v.at[j, k], wsem)
                for k, (src, jj) in enumerate(((wg_hbm, j_up), (wu_hbm, j_up), (wdT_hbm, j - 1)))]

        def start(copies):
            for cp in copies:
                cp.start()

        def wait(copies):
            for cp in copies:
                cp.wait()

        def wait_group(j):
            pltpu.make_async_copy(w_v.at[j], w_v.at[j], wsem).wait()

        def gate_up_weights(j, c):
            cs = slice(c * _GW, (c + 1) * _GW)
            return jnp.concatenate([w_v[j, 0, :, cs], w_v[j, 1, :, cs]], axis=1)

        def x_rows(r0, n, k0, k1):
            return pltpu.bitcast(x_v[r0 // 2:(r0 + n) // 2, k0:k1], bf16)

        def transpose_x(r0, n):
            x_v[r0 // 2:(r0 + n) // 2, :] = pltpu.bitcast(xT_v[:, r0:r0 + n].T, u32)

        def up(w, r0, n, c, vpu_tail=False):
            if vpu_tail:
                gu = jnp.dot(x_rows(r0, n, 0, KM), w[:KM], preferred_element_type=f32)
                gu = gu + tail_v[r0:r0 + n, 2 * _GW * c:2 * _GW * (c + 1)]
            else:
                gu = jnp.dot(x_rows(r0, n, 0, D), w, preferred_element_type=f32)
            h = _twice_geglu(gu[:, :_GW], gu[:, _GW:]).astype(bf16)
            h_v[r0 // 2:(r0 + n) // 2, c * _GW:(c + 1) * _GW] = pltpu.bitcast(h, u32)

        def down(wdT, r0, n):
            h = pltpu.bitcast(h_v[r0 // 2:(r0 + n) // 2, :], bf16)
            return lax.dot_general(wdT, h, (((1,), (1,)), ((), ())), preferred_element_type=f32)

        def broadcast_x_tail(r0):
            n = min(64, _RV - r0)
            if n > 0:
                xt = x_rows(r0, n, KM, D).astype(f32)
                for k in range(KT):
                    xb_v[k, r0:r0 + n, :] = jnp.broadcast_to(xt[:, k:k + 1], (n, 128))

        def tail_block(r0, c0, prev):
            acc = None
            if prev is not None:
                acc = pltpu.bitcast(pltpu.bitcast(prev, i32) & zero_v[...], f32)
            for k in range(KT):
                wk = wb_v[k, :, c0:c0 + 128]
                p = xb_v[k, r0:r0 + 16, :] * jnp.concatenate([wk, wk], axis=0)
                acc = p if acc is None else acc + p
            tail_v[r0:r0 + 16, c0:c0 + 128] = acc
            return acc

        def up0(r0, n, c):
            up(gate_up_weights(0, c), r0, n, c)

        x_copy(0).start()
        start(first_copies(0))
        acc_v[...] = jnp.zeros_like(acc_v)
        zero_v[...] = jnp.zeros_like(zero_v)
        x_copy(0).wait()
        x_copy(1).start()
        transpose_x(0, 256)
        wait(first_copies(0))
        start(first_copies(1))
        up0(0, 208, 0)

        x_copy(1).wait()
        x_copy(2).start()
        up0(208, 48, 0)
        for r0, n in ((256, 128), (384, 256)):
            transpose_x(r0, n)
            up0(r0, n, 0)

        wait(first_copies(1))
        x_copy(2).wait()
        x_copy(3).start()
        up0(0, 384, 1)
        transpose_x(640, 128)
        up0(640, 128, 0)
        up0(384, 256, 1)

        x_copy(3).wait()
        start(group_copies(1, 1))
        up0(640, 128, 1)
        transpose_x(768, 256)
        transpose_x(1024, 512)
        up0(768, 256, 0)
        broadcast_x_tail(0)
        up0(768, 256, 1)
        broadcast_x_tail(64)
        transpose_x(1536, 512)
        for i, (r0, c) in enumerate(((1024, 0), (1024, 1), (1536, 0), (1536, 1))):
            up0(r0, 512, c)
            broadcast_x_tail(128 * (i + 1))
            broadcast_x_tail(128 * (i + 1) + 64)

        def step(j, carry):
            wait_group(j)
            w = [gate_up_weights(j, c) for c in range(nc)]
            wdT = w_v[j, 2]
            for c in range(nc):
                wt = w[c][KM:].astype(f32)
                for k in range(KT):
                    wb_v[k, :, 2 * _GW * c:2 * _GW * (c + 1)] = jnp.broadcast_to(
                        wt[k:k + 1, :], (8, 2 * _GW))
            for i, r0 in enumerate([*range(_SM, S, _SM), 0]):
                acc_v[:, r0:r0 + _SM] += down(wdT, r0, _SM)
                if i == 0:
                    start(group_copies(j + 1, jnp.minimum(j + 1, nf - 1)))
                lo = max(r0, _RV)
                for c in range(nc):
                    up(w[c], lo, r0 + _SM - lo, c)
            prev = None
            for c in range(nc):
                for r0 in range(0, _RV, 16):
                    for c0 in range(2 * _GW * c, 2 * _GW * (c + 1), 128):
                        prev = tail_block(r0, c0, prev)
            for c in range(nc):
                up(w[c], 0, _RV, c, vpu_tail=True)
            return carry

        lax.fori_loop(1, nf, step, 0)

        wait_group(nf)
        out_copies = []
        for r0, n in _O_PIECES:
            y = acc_v[:, r0:r0 + n] + down(w_v[nf, 2], r0, n)
            o_v[:, r0:r0 + n] = (0.5 * y).astype(bf16)
            s = pl.ds(r0, n)
            out_copies.append(pltpu.make_async_copy(o_v.at[:, s], oT_hbm.at[:, s], osem))
            out_copies[-1].start()
        wait(out_copies)

    hbm = pl.BlockSpec(memory_space=pl.ANY)
    oT = pl.pallas_call(
        kernel,
        in_specs=[hbm] * 4,
        out_specs=hbm,
        out_shape=jax.ShapeDtypeStruct((D, S), bf16),
        scratch_shapes=[
            pltpu.VMEM((D, S), bf16),
            pltpu.VMEM((S // 2, D), u32),
            pltpu.VMEM((nf + 1, 3, D, _BF), bf16),
            pltpu.VMEM((S // 2, _BF), u32),
            pltpu.VMEM((D, S), f32),
            pltpu.VMEM((D, S), bf16),
            pltpu.VMEM((KT, _RV, 128), f32),
            pltpu.VMEM((KT, 8, 2 * _BF), f32),
            pltpu.VMEM((_RV, 2 * _BF), f32),
            pltpu.VMEM((16, 128), i32),
        ] + [pltpu.SemaphoreType.DMA] * 4,
        compiler_params=pltpu.CompilerParams(
            vmem_limit_bytes=100 * 1024 * 1024,
            disable_bounds_checks=True,
        ),
    )(x.reshape(S, D).T, w_gate, w_up, w_down.T)
    return oT.T.reshape(B, S0, D)
```
